```python
import os as _os
_os.environ.setdefault("JAX_PLATFORMS", "cpu")
import jax
import jax.numpy as jnp

def _softmax(x, axis=-1):
    return jax.nn.softmax(x, axis=axis)
def _gelu(x):
    return jax.nn.gelu(x, approximate=True)
def _silu(x):
    return jax.nn.silu(x)
def _sigmoid(x):
    return jax.nn.sigmoid(x)
def _layernorm(x, axis=-1, eps=1e-5):
    m = jnp.mean(x, axis=axis, keepdims=True)
    v = jnp.var(x, axis=axis, keepdims=True)
    return (x - m) / jnp.sqrt(v + eps)
def _scatter_add(tgt, idx, src, axis=0):
    return tgt.at[idx].add(src)
def _segment_sum(src, seg, n):
    return jax.ops.segment_sum(src, seg, n)
class _Rng:
    def __init__(self, key):
        self._k = key
    def _next(self):
        self._k, sub = jax.random.split(self._k)
        return sub
    def normal(self, shape):
        return jax.random.normal(self._next(), shape, dtype=jnp.bfloat16)
    def randint(self, lo, hi, shape):
        return jax.random.randint(self._next(), shape, lo, hi, dtype=jnp.int32)
    def uniform(self, shape, lo=0.0, hi=1.0):
        return jax.random.uniform(self._next(), shape, jnp.bfloat16, lo, hi)
    def permutation(self, n):
        return jax.random.permutation(self._next(), n)


kernel_name = 'concat_heads__mha_block_cached__mha_block_cached__near_ridge'

def setup_inputs():
    _rng = _Rng(jax.random.key(int.from_bytes(__import__("os").urandom(4), "little")))
    _w = (lambda a: (lambda t: t.astype(jnp.bfloat16) if jnp.issubdtype(t.dtype, jnp.floating) else t)(jnp.asarray(a)))
    def _A_setup():
        B, Sq, D = 32, 32, 640
        H, Sk, Dh = 32, 32, 128
        return {
            "x": _w((lambda *s: _rng.normal(s) * 0.8)(B, Sq, D)),
            "k_cache": _w((lambda *s: _rng.normal(s) * 0.8)(B, H, Sk, Dh)),
            "v_cache": _w((lambda *s: _rng.normal(s) * 0.05)(B, H, Sk, Dh)),
            "wq": _w((lambda *s: _rng.normal(s) * 0.8)(D, H * Dh) * (D ** -0.5)),
            "wo": _w((lambda *s: _rng.normal(s) * 0.05)(H * Dh, D) * ((H * Dh) ** -0.5)),
        }
    _A_in = _A_setup()

    def _B_setup():
        B, Sq, D = 32, 32, 640
        H, Sk, Dh = 32, 32, 128
        return {
            "x": _w((lambda *s: _rng.normal(s) * 0.8)(B, Sq, D)),
            "k_cache": _w((lambda *s: _rng.normal(s) * 0.8)(B, H, Sk, Dh)),
            "v_cache": _w((lambda *s: _rng.normal(s) * 0.05)(B, H, Sk, Dh)),
            "wq": _w((lambda *s: _rng.normal(s) * 0.8)(D, H * Dh) * (D ** -0.5)),
            "wo": _w((lambda *s: _rng.normal(s) * 0.05)(H * Dh, D) * ((H * Dh) ** -0.5)),
        }
    _B_in = _B_setup()

    return {
        "A_x": _A_in["x"],
        "A_k_cache": _A_in["k_cache"],
        "A_v_cache": _A_in["v_cache"],
        "A_wq": _A_in["wq"],
        "A_wo": _A_in["wo"],
        "B_x": _B_in["x"],
        "B_k_cache": _B_in["k_cache"],
        "B_v_cache": _B_in["v_cache"],
        "B_wq": _B_in["wq"],
        "B_wo": _B_in["wo"],
    }

def reference(A_x, A_k_cache, A_v_cache, A_wq, A_wo, B_x, B_k_cache, B_v_cache, B_wq, B_wo):
    def _A_ref(x, k_cache, v_cache, wq, wo):
        B, Sq, D = x.shape
        H, Dh = 32, 128
        q = (lambda x, *d: x.transpose(*d))((x @ wq).reshape(B, Sq, H, Dh), 0, 2, 1, 3)
        scores = jnp.einsum("bhqd,bhkd->bhqk", q, k_cache) * (Dh ** -0.5)
        p = _softmax(scores, axis=-1)
        o = jnp.einsum("bhqk,bhkd->bhqd", p, v_cache)
        return (lambda x, *d: x.transpose(*d))(o, 0, 2, 1, 3).reshape(B, Sq, H * Dh) @ wo

    def _B_ref(x, k_cache, v_cache, wq, wo):
        B, Sq, D = x.shape
        H, Dh = 32, 128
        q = (lambda x, *d: x.transpose(*d))((x @ wq).reshape(B, Sq, H, Dh), 0, 2, 1, 3)
        scores = jnp.einsum("bhqd,bhkd->bhqk", q, k_cache) * (Dh ** -0.5)
        p = _softmax(scores, axis=-1)
        o = jnp.einsum("bhqk,bhkd->bhqd", p, v_cache)
        return (lambda x, *d: x.transpose(*d))(o, 0, 2, 1, 3).reshape(B, Sq, H * Dh) @ wo

    a = _A_ref(A_x, A_k_cache, A_v_cache, A_wq, A_wo)
    b = _B_ref(B_x, B_k_cache, B_v_cache, B_wq, B_wo)
    return jnp.concatenate([a, b], axis=-1)
```

```python
import jax, jax.numpy as jnp
from jax import lax
import jax.experimental.pallas as pl
import jax.experimental.pallas.tpu as pltpu
import numpy as np, math, functools

F32 = jnp.float32; BF = jnp.bfloat16
CS = (128 ** -0.5) * math.log2(math.e)

def make(approx=True, skip='', nbc=True, issue_t=0, B0=16, XA=256, XB=512, LAG=2, EXTRA=0,
         order='kqpo', order_last='kop', order_first='kqpo', merge_ef=True, wq_split=False, osplit=False):
    NS = 16
    NOS = 4
    IDMA = 'idma' not in skip; ODMA = 'odma' not in skip

    def kernel(xA, kA, vA, wqA, woA, xB, kB, vB, wqB, woB, o_hbm,
               x_buf, k_buf, v_buf, wq_buf, wo_buf, acc, obuf, q_scr, o_scr, sems, xsem, s0, osem):
        srcs = ((xA, kA, vA, wqA, woA), (xB, kB, vB, wqB, woB))
        def rows(t): return pl.ds(t*128, 128)
        def cols(n): return pl.ds(n*128, 128)
        def cp_wq(slot, g, br, sem, n0=0, n1=4):
            wq = srcs[br][3]
            return [pltpu.make_async_copy(wq.at[:, pl.ds(g*512 + n0*128, (n1-n0)*128)], wq_buf.at[slot, :, pl.ds(n0*128, (n1-n0)*128)], sem)]
        def cp_wo(slot, g, br, sem):
            return [pltpu.make_async_copy(srcs[br][4].at[pl.ds(g*512, 512), :], wo_buf.at[slot], sem)]
        def cp_kv(which, slot, g, br, sem, b0=0, b1=32):
            src = srcs[br][which]; dst = k_buf if which == 1 else v_buf
            return [pltpu.make_async_copy(src.at[pl.ds(b0, b1-b0), pl.ds(g*4, 4)], dst.at[slot, pl.ds(b0, b1-b0)], sem)]
        def cp_x(br, sem, r0=0, r1=1024):
            return [pltpu.make_async_copy(srcs[br][0].at[pl.ds(r0, r1-r0), :], x_buf.at[br, pl.ds(r0, r1-r0)], sem)]
        def start(cps):
            for c in cps: c.start()
        def wait(cps):
            for c in cps: c.wait()
        def when(cond, f):
            if isinstance(cond, bool):
                if cond: f()
            else:
                pl.when(cond)(f)
        def kvo(i, br):
            g = i - 8 * br
            return cp_kv(1, i, g, br, sems.at[1, i]) + cp_kv(2, i, g, br, sems.at[2, i]) + cp_wo(i, g, br, sems.at[3, i])
        def start_chunk(i):
            if not IDMA: return
            when(i < 8, lambda: start(kvo(i, 0)))
            when((i >= 8) & (i < NS), lambda: start(kvo(i, 1)))
            when(i < 7, lambda: start(cp_wq(i + 1, i + 1, 0, sems.at[0, i + 1])))
            when((i >= 7) & (i < NS - 1), lambda: start(cp_wq(i + 1, i - 7, 1, sems.at[0, i + 1])))
            when(i == 7, lambda: start(cp_x(1, xsem.at[1])))
        def wait_chunk(i, kind):
            if not IDMA: return
            wait(cp_kv(1, i, 0, 0, sems.at[1, i])); wait(cp_kv(2, i, 0, 0, sems.at[2, i])); wait(cp_wo(i, 0, 0, sems.at[3, i]))
            if kind != 'last':
                wait(cp_wq(i + 1, 0, 0, sems.at[0, i + 1]))
                when(i == 7, lambda: wait(cp_x(1, xsem.at[1])))
        def cp_out(br, t, n=None):
            col = br * 640
            if n is None:
                return pltpu.make_async_copy(obuf.at[br, rows(t)], o_hbm.at[rows(t), pl.ds(col, 640)], osem.at[br, t])
            return pltpu.make_async_copy(obuf.at[br, rows(t), cols(n)], o_hbm.at[rows(t), pl.ds(col + n*128, 128)], osem.at[br, t])
        def out_start(br, t):
            if ODMA: cp_out(br, t).start()

        def P(cps): return cps if IDMA else []
        p_a = P(cp_x(0, s0.at[0], 0, XA) + cp_wq(0, 0, 0, s0.at[1], 0, 2 if wq_split else 4))
        p_a2 = P(cp_wq(0, 0, 0, s0.at[2], 2, 4) if wq_split else [])
        p_b = P(cp_x(0, s0.at[3], XA, XB))
        p_c = P(cp_x(0, s0.at[4], XB, 1024))
        p_d = P(cp_kv(1, 0, 0, 0, s0.at[5], 0, B0) + cp_wq(1, 1, 0, s0.at[6]) + cp_kv(2, 0, 0, 0, s0.at[7], 0, B0))
        p_e = P(cp_wo(0, 0, 0, s0.at[8]))
        p_f = P(cp_kv(1, 0, 0, 0, s0.at[9], B0, 32) + cp_kv(2, 0, 0, 0, s0.at[10], B0, 32)) if B0 < 32 else []
        for p in (p_a, p_a2, p_b, p_c, p_d, p_e, p_f): start(p)
        start_chunk(1)

        r = lax.broadcasted_iota(jnp.int32, (128, 128), 0) // 32
        c_ = lax.broadcasted_iota(jnp.int32, (128, 128), 1) // 32
        mask = r == c_

        def qproj(slot, br, t, qs, hooks=None):
            a = [None]*4
            for idx in range(20):
                n, kk = divmod(idx, 5)
                if hooks and idx in hooks: hooks[idx]()
                p = jnp.dot(x_buf[br, rows(t), cols(kk)], wq_buf[slot, rows(kk), cols(n)], preferred_element_type=F32)
                a[n] = p if kk == 0 else a[n] + p
                if kk == 4:
                    q_scr[qs, t, n] = a[n].astype(BF)
        def qk(slot, t, qs):
            ss = []
            for j in range(4):
                kt = k_buf[slot, pl.ds(4*t, 4), j].reshape(128, 128)
                ss.append(lax.dot_general(q_scr[qs, t, j], kt, (((1,), (1,)), ((), ())), preferred_element_type=F32))
            return ss
        def softmax(ss):
            es, ls = [], []
            for s in ss:
                s = jnp.where(mask, s, -1e30)
                m = jnp.max(s, axis=1, keepdims=True)
                e = jnp.exp2((s - m) * CS)
                l = jnp.sum(e, axis=1, keepdims=True)
                es.append(e.astype(BF)); ls.append(pl.reciprocal(l, approx=True) if approx else 1.0 / l)
            return es, ls
        def pv(slot, t, es, ls):
            for j in range(4):
                vt = v_buf[slot, pl.ds(4*t, 4), j].reshape(128, 128)
                o = jnp.dot(es[j], vt, preferred_element_type=F32) * ls[j]
                o_scr[t % NOS, j] = o.astype(BF)
        def outproj(slot, br, t, first=False, split=False):
            for n in range(5):
                a = None
                for j in range(4):
                    p = jnp.dot(o_scr[t % NOS, j], wo_buf[slot, rows(j), cols(n)], preferred_element_type=F32)
                    a = p if a is None else a + p
                y = a if first else acc[br, rows(t), cols(n)] + a
                if not split: acc[br, rows(t), cols(n)] = y
                obuf[br, rows(t), cols(n)] = y.astype(BF)
                if split and ODMA: cp_out(br, t, n).start()

        TB = B0 // 4
        def step(i, kind):
            br = i // 8
            nxt = i + 1; brn = nxt // 8
            prv = i - 1; brp = prv // 8
            if kind == 'first':
                wait(p_d)
            else:
                wait_chunk(i, kind)
            for t in range(8):
                st = {}
                def do_k():
                    if kind == 'first' and t == TB and not (merge_ef and TB <= LAG + 1): wait(p_f)
                    st['e'] = softmax(qk(i, t, i % 2))
                    if t == issue_t and kind != 'last':
                        start_chunk(i + 2)
                def do_o():
                    tt = t - LAG
                    if tt < 0:
                        if kind != 'first':
                            outproj(prv, brp, tt + 8)
                            when(i == 8 if kind == 'mid' else False, lambda: out_start(0, tt + 8))
                    else:
                        if tt == 0 and kind == 'first':
                            wait(p_e)
                            if merge_ef and TB <= LAG + 1: wait(p_f)
                        outproj(i, br, tt, first=(kind == 'first'))
                        if kind == 'last': out_start(1, tt)
                        elif kind == 'mid': when(i == 7, lambda: out_start(0, tt))
                def do_p():
                    pv(i, t, *st['e'])
                def do_q():
                    qproj(nxt, brn, t, nxt % 2)
                for ch in dict(first=order_first, mid=order, last=order_last)[kind]:
                    dict(k=do_k, o=do_o, p=do_p, q=do_q)[ch]()

        acc[1] = jnp.zeros((1024, 640), F32)
        for tt in range(8 - LAG, 8): acc[0, rows(tt)] = jnp.zeros((128, 640), F32)
        for t in range(8):
            if t == 0: wait(p_a)
            if t == XA // 128: wait(p_b)
            if t == XB // 128: wait(p_c)
            qproj(0, 0, t, 0, hooks={10: lambda: wait(p_a2)} if t == 0 else None)
        step(0, 'first')
        if EXTRA:
            def body2(i, carry):
                step(i % 14 + 1, 'mid'); return carry
            lax.fori_loop(0, NS - 2 + EXTRA, body2, 0)
        else:
            def body(i, carry):
                step(i, 'mid'); return carry
            lax.fori_loop(1, NS - 1, body, 0)
        step(NS - 1, 'last')
        for tt in range(8 - LAG, 8):
            sp = osplit and tt == 7
            outproj(NS - 1, 1, tt, split=sp)
            if not sp: out_start(1, tt)
        if ODMA:
            for b_ in range(2):
                for t in range(8): cp_out(b_, t).wait()

    @jax.jit
    def fn(A_x, A_k_cache, A_v_cache, A_wq, A_wo, B_x, B_k_cache, B_v_cache, B_wq, B_wo):
        anyspec = pl.BlockSpec(memory_space=pl.ANY)
        out = pl.pallas_call(
            kernel,
            in_specs=[anyspec]*10,
            out_specs=anyspec,
            out_shape=jax.ShapeDtypeStruct((1024, 1280), BF),
            scratch_shapes=[
                pltpu.VMEM((2, 1024, 640), BF),
                pltpu.VMEM((NS, 32, 4, 32, 128), BF),
                pltpu.VMEM((NS, 32, 4, 32, 128), BF),
                pltpu.VMEM((NS, 640, 512), BF),
                pltpu.VMEM((NS, 512, 640), BF),
                pltpu.VMEM((2, 1024, 640), F32),
                pltpu.VMEM((2, 1024, 640), BF),
                pltpu.VMEM((2, 8, 4, 128, 128), BF),
                pltpu.VMEM((NOS, 4, 128, 128), BF),
                pltpu.SemaphoreType.DMA((4, NS)),
                pltpu.SemaphoreType.DMA((2,)),
                pltpu.SemaphoreType.DMA((11,)),
                pltpu.SemaphoreType.DMA((2, 8)),
            ],
            compiler_params=pltpu.CompilerParams(vmem_limit_bytes=100*1024*1024, disable_bounds_checks=nbc),
        )(A_x.reshape(1024, 640), A_k_cache, A_v_cache, A_wq, A_wo, B_x.reshape(1024, 640), B_k_cache, B_v_cache, B_wq, B_wo)
        return out.reshape(32, 32, 1280)
    return fn
pallas_concat_heads__mha_block_cached__mha_block_cached__near_ridge_kernel = make(osplit=True)
```

```python
import jax, jax.numpy as jnp
from jax import lax
import jax.experimental.pallas as pl
import jax.experimental.pallas.tpu as pltpu
import numpy as np, math, functools

F32 = jnp.float32; BF = jnp.bfloat16
CS = (128 ** -0.5) * math.log2(math.e)

def make(approx='n', skip='', nbc=True, issue_t=0, B0=16, XS=(128, 256, 512, 768), LAG=4, EXTRA=0,
         order='okqp', order_last='kop', order_first=None, osplit=True, pairs=True, scopes=False,
         merge_ef=True, merge_wb=False, zero_at=-1, late_issue=0, flags={'XLA_TPU_RESCHEDULE_DMA_DONES': True}, ninf=True, unroll=2):
    NS = 16
    NOS = 4 if LAG <= 3 else 8
    order_first = order_first or order
    IDMA = 'idma' not in skip and 'sdma' not in skip; PDMA = 'idma' not in skip and 'pdma' not in skip; ODMA = 'odma' not in skip
    xb = (0,) + tuple(XS) + (1024,)
    NX = len(xb) - 1
    assert all(v % 128 == 0 for v in xb)

    def kernel(xA, kA, vA, wqA, woA, xB, kB, vB, wqB, woB, o_hbm,
               x_buf, k_buf, v_buf, wq_buf, wo_buf, acc, obuf, q_scr, o_scr, sems, s0, osem):
        srcs = ((xA, kA, vA, wqA, woA), (xB, kB, vB, wqB, woB))
        def rows(t): return pl.ds(t*128, 128)
        def cols(n): return pl.ds(n*128, 128)
        def shr(i, n): return i >> n if isinstance(i, int) else lax.shift_right_logical(i, jnp.int32(n))
        def cp_wq(slot, g, br, sem, n0=0, n1=4):
            wq = srcs[br][3]
            return [pltpu.make_async_copy(wq.at[:, pl.ds(g*512 + n0*128, (n1-n0)*128)], wq_buf.at[slot, :, pl.ds(n0*128, (n1-n0)*128)], sem)]
        def cp_wo(slot, g, br, sem):
            return [pltpu.make_async_copy(srcs[br][4].at[pl.ds(g*512, 512), :], wo_buf.at[slot], sem)]
        def cp_kv(which, slot, g, br, sem, b0=0, b1=32):
            src = srcs[br][which]; dst = k_buf if which == 1 else v_buf
            return [pltpu.make_async_copy(src.at[pl.ds(b0, b1-b0), pl.ds(g*4, 4)], dst.at[slot, pl.ds(b0, b1-b0)], sem)]
        def cp_x(br, sem, r0=0, r1=1024):
            return [pltpu.make_async_copy(srcs[br][0].at[pl.ds(r0, r1-r0), :], x_buf.at[br, pl.ds(r0, r1-r0)], sem)]
        def start(cps):
            for c in cps: c.start()
        wcount = [0]
        def wait(cps):
            if not cps: return
            if scopes:
                wcount[0] += 1
                with jax.named_scope('w%02d' % wcount[0]):
                    for c in cps: c.wait()
            else:
                for c in cps: c.wait()
        def when(cond, f):
            if isinstance(cond, bool):
                if cond: f()
            else:
                pl.when(cond)(f)
        def kvo(i, br):
            g = i - 8 * br; sem = sems.at[i & 1]
            return cp_kv(1, i, g, br, sem) + cp_kv(2, i, g, br, sem) + cp_wo(i, g, br, sem)
        def start_chunk(i):
            if not IDMA: return
            j = i + 1; sem = sems.at[i & 1]
            when(i < 8, lambda: start(kvo(i, 0)))
            when((i >= 8) & (i < NS), lambda: start(kvo(i, 1)))
            when(j < 8, lambda: start(cp_wq(j, j, 0, sem)))
            when((j >= 8) & (j < NS), lambda: start(cp_wq(j, j - 8, 1, sem)))
            when(i == 7, lambda: start(cp_x(1, sem)))
        def wait_chunk(i, has_q):
            if not IDMA: return
            sem = sems.at[i & 1]
            cps = cp_kv(1, i, 0, 0, sem) + cp_kv(2, i, 0, 0, sem) + cp_wo(i, 0, 0, sem)
            if has_q: cps = cps + cp_wq(i + 1, 0, 0, sem)
            wait(cps)
            if has_q: when(i == 7, lambda: wait(cp_x(1, sem)))
        def cp_out(br, t, n=None):
            col = br * 640
            if n is None:
                return pltpu.make_async_copy(obuf.at[br, rows(t)], o_hbm.at[rows(t), pl.ds(col, 640)], osem.at[0])
            return pltpu.make_async_copy(obuf.at[br, rows(t), cols(n)], o_hbm.at[rows(t), pl.ds(col + n*128, 128)], osem.at[0])
        def out_start(br, t):
            if ODMA: cp_out(br, t).start()

        def P(cps): return cps if PDMA else []
        p_x = [P(cp_x(0, s0.at[k], xb[k], xb[k+1])) for k in range(NX)]
        p_w0 = P(cp_wq(0, 0, 0, s0.at[0], 0, 2 if pairs else 4))
        p_w0b = P(cp_wq(0, 0, 0, s0.at[NX - 1 if merge_wb else NX], 2, 4)) if pairs else []
        p_d = P(cp_kv(1, 0, 0, 0, s0.at[NX+1], 0, B0) + cp_wq(1, 1, 0, s0.at[NX+1]) + cp_kv(2, 0, 0, 0, s0.at[NX+1], 0, B0))
        p_e = P(cp_wo(0, 0, 0, s0.at[NX+2]))
        p_f = P(cp_kv(1, 0, 0, 0, s0.at[NX+2 if merge_ef else NX+3], B0, 32) + cp_kv(2, 0, 0, 0, s0.at[NX+2 if merge_ef else NX+3], B0, 32)) if B0 < 32 else []
        seq = [p_x[0], p_w0] + p_x[1:] + [p_w0b, p_d, p_e, p_f]
        nfirst = len(seq) if not late_issue else late_issue
        for p in seq[:nfirst]: start(p)
        if not late_issue: start_chunk(1)

        r = lax.broadcasted_iota(jnp.int32, (128, 128), 0) // 32
        c_ = lax.broadcasted_iota(jnp.int32, (128, 128), 1) // 32
        mask = r == c_

        def qproj(slot, br, t, qs, n0=0, n1=4):
            a = [None]*4
            for n in range(n0, n1):
                for kk in range(5):
                    p = jnp.dot(x_buf[br, rows(t), cols(kk)], wq_buf[slot, rows(kk), cols(n)], preferred_element_type=F32)
                    a[n] = p if kk == 0 else a[n] + p
                q_scr[qs, t, n] = a[n].astype(BF)
        def qk(slot, t, qs):
            ss = []
            for j in range(4):
                kt = k_buf[slot, pl.ds(4*t, 4), j].reshape(128, 128)
                ss.append(lax.dot_general(q_scr[qs, t, j], kt, (((1,), (1,)), ((), ())), preferred_element_type=F32))
            return ss
        def softmax(ss):
            es, ls = [], []
            for s in ss:
                s = jnp.where(mask, s, -jnp.inf if ninf else -1e30)
                m = jnp.max(s, axis=1, keepdims=True)
                e = jnp.exp2((s - m) * CS)
                l = jnp.sum(e, axis=1, keepdims=True)
                if approx == 'n':
                    r0 = pl.reciprocal(l, approx=True)
                    rl = r0 * (2.0 - l * r0)
                else:
                    rl = pl.reciprocal(l, approx=True) if approx else 1.0 / l
                es.append(e.astype(BF)); ls.append(rl)
            return es, ls
        def pv(slot, t, es, ls):
            for j in range(4):
                vt = v_buf[slot, pl.ds(4*t, 4), j].reshape(128, 128)
                o = jnp.dot(es[j], vt, preferred_element_type=F32) * ls[j]
                o_scr[t % NOS, j] = o.astype(BF)
        def outproj(slot, br, t, first=False, split=False):
            for n in range(5):
                a = None
                for j in range(4):
                    p = jnp.dot(o_scr[t % NOS, j], wo_buf[slot, rows(j), cols(n)], preferred_element_type=F32)
                    a = p if a is None else a + p
                y = a if first else acc[br, rows(t), cols(n)] + a
                if not split: acc[br, rows(t), cols(n)] = y
                obuf[br, rows(t), cols(n)] = y.astype(BF)
                if split and ODMA: cp_out(br, t, n).start()

        TB = B0 // 4
        assert not merge_ef or LAG == TB
        def step(i, kind):
            br = shr(i, 3)
            nxt = i + 1; brn = shr(nxt, 3)
            prv = i - 1; brp = shr(prv, 3)
            if kind == 'first': wait(p_d)
            else: wait_chunk(i, kind != 'last')
            for t in range(8):
                st = {}
                def do_k():
                    if kind == 'first' and t == TB and not merge_ef: wait(p_f)
                    st['e'] = softmax(qk(i, t, i & 1))
                    if t == issue_t and kind != 'last':
                        start_chunk(i + 2)
                def do_o():
                    tt = t - LAG
                    if tt < 0:
                        if kind != 'first':
                            outproj(prv, brp, tt + 8)
                            when(i == 8 if kind == 'mid' else False, lambda: out_start(0, tt + 8))
                    else:
                        if tt == 0 and kind == 'first':
                            wait(p_e + (p_f if merge_ef else []))
                        outproj(i, br, tt, first=(kind == 'first'))
                        if kind == 'last': out_start(1, tt)
                        elif kind == 'mid': when(i == 7, lambda: out_start(0, tt))
                def do_p():
                    pv(i, t, *st['e'])
                def do_q():
                    qproj(nxt, brn, t, nxt & 1)
                for ch in dict(first=order_first, mid=order, last=order_last)[kind]:
                    dict(k=do_k, o=do_o, p=do_p, q=do_q)[ch]()

        def zero_acc():
            acc[1] = jnp.zeros((1024, 640), F32)
            for tt in range(8 - LAG, 8): acc[0, rows(tt)] = jnp.zeros((128, 640), F32)
        if zero_at < 0: zero_acc()
        for t in range(8):
            for k in range(NX):
                if t * 128 == xb[k]:
                    wait(p_x[k] + (p_w0 if k == 0 else []) + (p_w0b if (k == NX - 1 and merge_wb) else []))
                    if k == 0 and late_issue:
                        for p in seq[nfirst:]: start(p)
                        start_chunk(1)
                    if k == zero_at: zero_acc()
            qproj(0, 0, t, 0, 0, 2 if pairs else 4)
        if pairs:
            if not merge_wb: wait(p_w0b)
            for t in range(8): qproj(0, 0, t, 0, 2, 4)
        step(0, 'first')
        if EXTRA:
            def body2(i, carry):
                step(i % 8 + 1, 'mid'); return carry
            lax.fori_loop(0, NS - 2 + EXTRA, body2, 0)
        else:
            def body(i, carry):
                step(i, 'mid'); return carry
            lax.fori_loop(1, NS - 1, body, 0, unroll=unroll)
        step(NS - 1, 'last')
        for tt in range(8 - LAG, 8):
            sp = osplit and tt == 7
            outproj(NS - 1, 1, tt, split=sp)
            if not sp: out_start(1, tt)
        if ODMA:
            wait([pltpu.make_async_copy(obuf, obuf, osem.at[0])])

    @jax.jit
    def fn(A_x, A_k_cache, A_v_cache, A_wq, A_wo, B_x, B_k_cache, B_v_cache, B_wq, B_wo):
        anyspec = pl.BlockSpec(memory_space=pl.ANY)
        out = pl.pallas_call(
            kernel,
            in_specs=[anyspec]*10,
            out_specs=anyspec,
            out_shape=jax.ShapeDtypeStruct((1024, 1280), BF),
            scratch_shapes=[
                pltpu.VMEM((2, 1024, 640), BF),
                pltpu.VMEM((NS, 32, 4, 32, 128), BF),
                pltpu.VMEM((NS, 32, 4, 32, 128), BF),
                pltpu.VMEM((NS, 640, 512), BF),
                pltpu.VMEM((NS, 512, 640), BF),
                pltpu.VMEM((2, 1024, 640), F32),
                pltpu.VMEM((2, 1024, 640), BF),
                pltpu.VMEM((2, 8, 4, 128, 128), BF),
                pltpu.VMEM((NOS, 4, 128, 128), BF),
                pltpu.SemaphoreType.DMA((2,)),
                pltpu.SemaphoreType.DMA((NX + (3 if merge_ef else 4),)),
                pltpu.SemaphoreType.DMA((1,)),
            ],
            compiler_params=pltpu.CompilerParams(vmem_limit_bytes=100*1024*1024, disable_bounds_checks=nbc, flags=flags),
        )(A_x.reshape(1024, 640), A_k_cache, A_v_cache, A_wq, A_wo, B_x.reshape(1024, 640), B_k_cache, B_v_cache, B_wq, B_wo)
        return out.reshape(32, 32, 1280)
    return fn
pallas_concat_heads__mha_block_cached__mha_block_cached__near_ridge_kernel = make()
```

```python
import math

import jax
import jax.numpy as jnp
from jax import lax
import jax.experimental.pallas as pl
import jax.experimental.pallas.tpu as pltpu

F32 = jnp.float32
BF16 = jnp.bfloat16

M, D = 1024, 640
NS = 16
NT = 8
LAG = 4
BH = 4 * LAG
CS = (128 ** -0.5) * math.log2(math.e)
FIRST_Q = (("x0+w0-1"), ("x1"), ("w2"), ("x2"), ("w3"), ("x3"), ("x4-5"), ("x6-7"))
FIRST_KV = (0, 8, 16, 24, 32)


def _kernel(xA, kA, vA, wqA, woA, xB, kB, vB, wqB, woB, o_hbm,
            x_buf, k_buf, v_buf, wq_buf, wo_buf, acc, obuf, q_scr, o_scr, sems, sem0, osem):
    srcs = ((xA, kA, vA, wqA, woA), (xB, kB, vB, wqB, woB))

    def rows(t):
        return pl.ds(t * 128, 128)

    def cols(n):
        return pl.ds(n * 128, 128)

    def branch_of(i):
        return i >> 3 if isinstance(i, int) else lax.shift_right_logical(i, jnp.int32(3))

    def when(cond, f):
        if isinstance(cond, bool):
            if cond:
                f()
        else:
            pl.when(cond)(f)

    def cp_x(br, sem, t0=0, t1=NT):
        r = pl.ds(t0 * 128, (t1 - t0) * 128)
        return [pltpu.make_async_copy(srcs[br][0].at[r, :], x_buf.at[br, r], sem)]

    def cp_kv(which, slot, g, br, sem, b0, b1):
        dst = k_buf if which == 1 else v_buf
        b = pl.ds(b0, b1 - b0)
        return [pltpu.make_async_copy(srcs[br][which].at[b, pl.ds(g * 4, 4)], dst.at[slot, b], sem)]

    def cp_wq(slot, g, br, sem, n0=0, n1=4):
        w = (n1 - n0) * 128
        return [pltpu.make_async_copy(srcs[br][3].at[:, pl.ds(g * 512 + n0 * 128, w)],
                                      wq_buf.at[slot, :, pl.ds(n0 * 128, w)], sem)]

    def cp_wo(slot, g, br, sem):
        return [pltpu.make_async_copy(srcs[br][4].at[pl.ds(g * 512, 512), :], wo_buf.at[slot], sem)]

    def start(cps):
        for c in cps:
            c.start()

    def wait(cps):
        for c in cps:
            c.wait()

    def sem_a(i):
        return sems.at[i & 1]

    def sem_b(i):
        return sems.at[2 + (i & 1)]

    def part_a(i, g, br, has_q, gq, brq):
        s = sem_a(i)
        return (cp_kv(1, i, g, br, s, 0, BH) + (cp_wq(i + 1, gq, brq, s) if has_q else [])
                + cp_kv(2, i, g, br, s, 0, BH))

    def part_b(i, g, br):
        s = sem_b(i)
        return cp_wo(i, g, br, s) + cp_kv(1, i, g, br, s, BH, 32) + cp_kv(2, i, g, br, s, BH, 32)

    def start_a(i):
        when(i < 7, lambda: start(part_a(i, i, 0, True, i + 1, 0)))
        when(i == 7, lambda: start(part_a(i, 7, 0, True, 0, 1) + cp_x(1, sem_a(i))))
        when((i >= 8) & (i < NS - 1), lambda: start(part_a(i, i - 8, 1, True, i - 7, 1)))
        when(i == NS - 1, lambda: start(part_a(i, 7, 1, False, 0, 0)))

    def start_b(i):
        when(i < 8, lambda: start(part_b(i, i, 0)))
        when((i >= 8) & (i < NS), lambda: start(part_b(i, i - 8, 1)))

    def wait_a(i, has_q):
        wait(part_a(i, 0, 0, has_q, 0, 0))
        if has_q:
            when(i == 7, lambda: wait(cp_x(1, sem_a(i))))

    def wait_b(i):
        wait(part_b(i, 0, 0))

    def out_start(br, t, n=None):
        c = pl.ds(br * D, D) if n is None else pl.ds(br * D + n * 128, 128)
        src = obuf.at[br, rows(t)] if n is None else obuf.at[br, rows(t), cols(n)]
        pltpu.make_async_copy(src, o_hbm.at[rows(t), c], osem.at[0]).start()

    first_q = []
    for k, item in enumerate(FIRST_Q):
        cps = []
        for it in item.split("+"):
            lo, hi = int(it[1]), int(it[-1]) + 1
            cps += cp_x(0, sem0.at[k], lo, hi) if it[0] == "x" else cp_wq(0, 0, 0, sem0.at[k], lo, hi)
        first_q.append(cps)
    first_kv = []
    for k in range(len(FIRST_KV) - 1):
        s = sem0.at[len(FIRST_Q) + k]
        b0, b1 = FIRST_KV[k], FIRST_KV[k + 1]
        cps = cp_kv(1, 0, 0, 0, s, b0, b1)
        if b0 == 0:
            cps = cps + cp_wq(1, 1, 0, s)
        if b0 == BH:
            cps = cp_wo(0, 0, 0, s) + cps
        first_kv.append(cps + cp_kv(2, 0, 0, 0, s, b0, b1))
    for cps in first_q + first_kv:
        start(cps)
    start_a(1)
    start_b(1)

    r_id = lax.broadcasted_iota(jnp.int32, (128, 128), 0) // 32
    c_id = lax.broadcasted_iota(jnp.int32, (128, 128), 1) // 32
    mask = r_id == c_id

    def stage_q(slot, br, t, n0=0, n1=4):
        for n in range(n0, n1):
            a = None
            for kk in range(D // 128):
                p = jnp.dot(x_buf[br, rows(t), cols(kk)], wq_buf[slot, rows(kk), cols(n)],
                            preferred_element_type=F32)
                a = p if a is None else a + p
            q_scr[slot & 1, t, n] = a.astype(BF16)

    def stage_k(slot, t):
        ss = []
        for j in range(4):
            kt = k_buf[slot, pl.ds(4 * t, 4), j].reshape(128, 128)
            ss.append(lax.dot_general(q_scr[slot & 1, t, j], kt, (((1,), (1,)), ((), ())),
                                      preferred_element_type=F32))
        es, rs = [], []
        for s in ss:
            s = jnp.where(mask, s, -jnp.inf)
            m = jnp.max(s, axis=1, keepdims=True)
            e = jnp.exp2((s - m) * CS)
            l = jnp.sum(e, axis=1, keepdims=True)
            rl = pl.reciprocal(l, approx=True)
            rl = rl * (2.0 - l * rl)
            es.append(e.astype(BF16))
            rs.append(rl)
        return es, rs

    def stage_p(slot, t, es, rs):
        for j in range(4):
            vt = v_buf[slot, pl.ds(4 * t, 4), j].reshape(128, 128)
            o = jnp.dot(es[j], vt, preferred_element_type=F32) * rs[j]
            o_scr[t, j] = o.astype(BF16)

    def stage_o(slot, br, t, first, tail=False):
        for n in range(D // 128):
            a = None
            for j in range(4):
                p = jnp.dot(o_scr[t, j], wo_buf[slot, rows(j), cols(n)], preferred_element_type=F32)
                a = p if a is None else a + p
            if first is True:
                y = a
            elif first is False:
                y = acc[br, rows(t), cols(n)] + a
            else:
                y = jnp.where(first, a, acc[br, rows(t), cols(n)] + a)
            if not tail:
                acc[br, rows(t), cols(n)] = y
            obuf[br, rows(t), cols(n)] = y.astype(BF16)
            if tail:
                out_start(br, t, n)

    def step(i, kind):
        br = branch_of(i)
        nxt, prv = i + 1, i - 1
        for t in range(NT):
            if kind == "first":
                if 4 * t in FIRST_KV:
                    wait(first_kv[FIRST_KV.index(4 * t)])
            elif t == 0:
                wait_a(i, kind != "last")
            elif t == LAG:
                wait_b(i)

            def do_o():
                if t < LAG:
                    if kind == "mid":
                        stage_o(prv, branch_of(prv), t - LAG + NT, (prv & 7) == 0)
                        pl.when(i == 8)(lambda: out_start(0, t - LAG + NT))
                    elif kind == "last":
                        stage_o(prv, 1, t - LAG + NT, False)
                elif kind == "mid":
                    stage_o(i, br, t - LAG, i == 8)
                    pl.when(i == 7)(lambda: out_start(0, t - LAG))
                else:
                    stage_o(i, br, t - LAG, kind == "first")
                    if kind == "last":
                        out_start(1, t - LAG)

            if kind != "last":
                do_o()
            es, rs = stage_k(i, t)
            if kind != "last":
                if t == 0:
                    start_a(i + 2)
                if t == LAG:
                    start_b(i + 2)
                stage_q(nxt, branch_of(nxt), t)
            else:
                do_o()
            stage_p(i, t, es, rs)

    have_x, have_w, done = set(), set(), set()
    for k, item in enumerate(FIRST_Q):
        wait(first_q[k])
        for it in item.split("+"):
            (have_x if it[0] == "x" else have_w).update(range(int(it[1]), int(it[-1]) + 1))
        for t in sorted(have_x):
            for n in sorted(have_w):
                if (t, n) not in done:
                    done.add((t, n))
                    stage_q(0, 0, t, n, n + 1)

    step(0, "first")

    def body(i, carry):
        step(i, "mid")
        return carry

    lax.fori_loop(1, NS - 1, body, 0, unroll=2)
    step(NS - 1, "last")
    for t in range(NT - LAG, NT):
        stage_o(NS - 1, 1, t, False, tail=(t == NT - 1))
        if t != NT - 1:
            out_start(1, t)
    pltpu.make_async_copy(obuf, obuf, osem.at[0]).wait()


@jax.jit
def pallas_concat_heads__mha_block_cached__mha_block_cached__near_ridge_kernel(
    A_x: jax.Array,
    A_k_cache: jax.Array,
    A_v_cache: jax.Array,
    A_wq: jax.Array,
    A_wo: jax.Array,
    B_x: jax.Array,
    B_k_cache: jax.Array,
    B_v_cache: jax.Array,
    B_wq: jax.Array,
    B_wo: jax.Array,
):
    hbm = pl.BlockSpec(memory_space=pl.ANY)
    out = pl.pallas_call(
        _kernel,
        in_specs=[hbm] * 10,
        out_specs=hbm,
        out_shape=jax.ShapeDtypeStruct((M, 2 * D), BF16),
        scratch_shapes=[
            pltpu.VMEM((2, M, D), BF16),
            pltpu.VMEM((NS, 32, 4, 32, 128), BF16),
            pltpu.VMEM((NS, 32, 4, 32, 128), BF16),
            pltpu.VMEM((NS, D, 512), BF16),
            pltpu.VMEM((NS, 512, D), BF16),
            pltpu.VMEM((2, M, D), F32),
            pltpu.VMEM((2, M, D), BF16),
            pltpu.VMEM((2, NT, 4, 128, 128), BF16),
            pltpu.VMEM((NT, 4, 128, 128), BF16),
            pltpu.SemaphoreType.DMA((4,)),
            pltpu.SemaphoreType.DMA((len(FIRST_Q) + len(FIRST_KV) - 1,)),
            pltpu.SemaphoreType.DMA((1,)),
        ],
        compiler_params=pltpu.CompilerParams(
            vmem_limit_bytes=100 * 1024 * 1024,
            disable_bounds_checks=True,
            flags={"XLA_TPU_RESCHEDULE_DMA_DONES": True},
        ),
    )(A_x.reshape(M, D), A_k_cache, A_v_cache, A_wq, A_wo,
      B_x.reshape(M, D), B_k_cache, B_v_cache, B_wq, B_wo)
    return out.reshape(32, 32, 2 * D)
```
